```python
import os as _os
_os.environ.setdefault("JAX_PLATFORMS", "cpu")
import jax
import jax.numpy as jnp

def _softmax(x, axis=-1):
    return jax.nn.softmax(x, axis=axis)
def _gelu(x):
    return jax.nn.gelu(x, approximate=True)
def _silu(x):
    return jax.nn.silu(x)
def _sigmoid(x):
    return jax.nn.sigmoid(x)
def _layernorm(x, axis=-1, eps=1e-5):
    m = jnp.mean(x, axis=axis, keepdims=True)
    v = jnp.var(x, axis=axis, keepdims=True)
    return (x - m) / jnp.sqrt(v + eps)
def _scatter_add(tgt, idx, src, axis=0):
    return tgt.at[idx].add(src)
def _segment_sum(src, seg, n):
    return jax.ops.segment_sum(src, seg, n)
class _Rng:
    def __init__(self, key):
        self._k = key
    def _next(self):
        self._k, sub = jax.random.split(self._k)
        return sub
    def normal(self, shape):
        return jax.random.normal(self._next(), shape, dtype=jnp.bfloat16)
    def randint(self, lo, hi, shape):
        return jax.random.randint(self._next(), shape, lo, hi, dtype=jnp.int32)
    def uniform(self, shape, lo=0.0, hi=1.0):
        return jax.random.uniform(self._next(), shape, jnp.bfloat16, lo, hi)
    def permutation(self, n):
        return jax.random.permutation(self._next(), n)


kernel_name = 'standalone__dense_activation_silu__prompt'

def setup_inputs():
    _rng = _Rng(jax.random.key(int.from_bytes(__import__("os").urandom(4), "little")))
    _w = (lambda a: (lambda t: t.astype(jnp.bfloat16) if jnp.issubdtype(t.dtype, jnp.floating) else t)(jnp.asarray(a)))
    B, S, D, F = 1, 2048, 448, 1792
    return {
        "x": _w((lambda *s: _rng.normal(s) * 0.05)(B, S, D)),
        "w1": _w((lambda *s: _rng.normal(s) * 0.05)(D, F) * (D ** -0.5)),
        "w2": _w((lambda *s: _rng.normal(s) * 0.05)(F, D) * (F ** -0.5)),
    }

def reference(x, w1, w2):
    h = jnp.einsum("bsd,df->bsf", x, w1)
    h = _silu(h)
    out = jnp.einsum("bsf,fd->bsd", h, w2)
    return out
```

```python
import jax
import jax.numpy as jnp
from jax import lax
import jax.experimental.pallas as pl
import jax.experimental.pallas.tpu as pltpu

D, F, M = 448, 1792, 2048
bf = jnp.bfloat16
PAD = 16

def silu_bf16(h):
    hh = 0.5 * h
    return (hh + hh * jnp.tanh(hh)).astype(bf)

def make(first=(512, 512), ks=(128, 128, 128, 64), lkx=380, lkw=240, grow="w256 w256 w768", xrest=(512, 1024), mb=512, m2=(512, 512, 512, 256), last=(384, 64),
         lw=240, lx=520, l2=4000, lxr=2000, flags={'XLA_TPU_RESCHEDULE_DMA_DONES': True}, ahead=100, scoped=False, pin0=(0, 0)):
    stages = []
    m0, c0 = first
    nk = len(ks)
    assert sum(ks) == D
    ko = [sum(ks[:i]) for i in range(nk)]
    pos = {"x": m0, "w": c0}
    for st in grow.split():
        cur = []
        for p in st.split("+"):
            k, n = p[0], int(p[1:])
            cur.append((k, pos[k], n)); pos[k] += n
        stages.append(cur)
    assert pos["w"] == F
    ngrow = len(stages)
    for n in xrest:
        stages.append([("x", pos["x"], n)]); pos["x"] += n
    assert pos["x"] == M, pos
    ns = len(stages)
    def split(lo, hi):
        n = -(-(hi - lo) // mb)
        q = (hi - lo) // 128
        e = [lo + (q * i // n) * 128 for i in range(n + 1)]
        return list(zip(e[:-1], e[1:]))
    items, need = [], []
    hx, hw = m0, c0
    for st in stages:
        need.append(len(items))
        nw = sum(p[2] for p in st if p[0] == "w")
        if nw and hx:
            for a, b in split(0, hx):
                items.append((a, b, hw, hw + nw))
        hw += nw
        for k, o, n in st:
            if k == "x":
                if hw:
                    for a, b in split(o, o + n):
                        items.append((a, b, 0, hw))
                hx += n
    need.append(len(items))
    last_k = m0 * c0 // 512
    start = [0]
    for (r0, r1, f0, f1) in items:
        start.append(start[-1] + (r1 - r0) * (f1 - f0) // 128)
    place = {}
    prev = (-1, 0)
    for s in range(ns + 1):
        if s == ns:
            lead = l2
        elif s >= ngrow:
            lead = lxr
        else:
            lead = lx if any(p[0] == "x" for p in stages[s]) else lw
        t = start[need[s]] - lead
        if t < 0:
            key = (-1, max(0, last_k + t))
        else:
            i = max(j for j in range(need[s]) if start[j] <= t)
            key = (i, t - start[i])
        key = max(key, prev); prev = key
        place.setdefault(key[0], []).append((s, key[1]))
    outs = []
    q0 = 0
    for m in m2:
        outs.append((q0, q0 + m, 0, D)); q0 += m
    if q0 < M:
        r0 = 0
        for r in last:
            outs.append((q0, M, r0, r0 + r)); r0 += r
        assert r0 == D
    no = len(outs)
    xpieces = [p for st in stages for p in st if p[0] == "x"]

    def kern(xT_hbm, w1_hbm, w2T_hbm, oT_hbm, x_v, w1_v, w2_v, a_v, *sc):
        o_v = sc[:no]
        sem_out = sc[no]
        def phase1(sem_in):
            def cp(s, piece):
                k, o, n = piece
                src, dst = (xT_hbm, x_v) if k == "x" else (w1_hbm, w1_v)
                return pltpu.make_async_copy(src.at[:, pl.ds(o, n)], dst.at[pl.ds(0, D), pl.ds(o, n)], sem_in.at[s])
            cps = [[cp(s, p) for p in st] for s, st in enumerate(stages)]
            cps.append([pltpu.make_async_copy(w2T_hbm, w2_v.at[pl.ds(0, D)], sem_in.at[ns])])
            kx = [pltpu.make_async_copy(xT_hbm.at[pl.ds(ko[i], ks[i]), pl.ds(0, m0)], x_v.at[pl.ds(ko[i], ks[i]), pl.ds(0, m0)],
                                        sem_in.at[ns + 1 + 2 * i]) for i in range(nk)]
            kw = [pltpu.make_async_copy(w1_hbm.at[pl.ds(ko[i], ks[i]), pl.ds(0, c0)], w1_v.at[pl.ds(ko[i], ks[i]), pl.ds(0, c0)],
                                        sem_in.at[ns + 2 + 2 * i]) for i in range(nk)]
            queue = [c for i in range(nk) for c in (kx[i], kw[i])] + [c for st in cps for c in st]
            def issue(n):
                for _ in range(min(n, len(queue))):
                    queue.pop(0).start()
            issue(ahead)
            xt = {}
            def xrows(r0, r1):
                for r in range(r0, r1, 128):
                    if r not in xt:
                        _, o, n = [p for p in xpieces if p[1] <= r < p[1] + p[2]][0]
                        n = min(o + n - r, r1 - r)
                        v = x_v[0:D, r:r + n].T
                        for q in range(0, n, 128):
                            xt[r + q] = v[q:q + 128]
                vs = [xt[r] for r in range(r0, r1, 128)]
                return vs[0] if len(vs) == 1 else jnp.concatenate(vs, axis=0)
            def wait(s, pinval):
                if pinval is not None:
                    bufs = [w2_v] if s == ns else [x_v if k == "x" else w1_v for k in sorted(set(p[0] for p in stages[s]))]
                    for b in bufs:
                        b[D:D + PAD, 0:pinval.shape[1]] = pinval
                for c in cps[s]:
                    c.wait()
                issue(len(cps[s]))
            def pin(buf, val):
                buf[D:D + PAD, 0:val.shape[1]] = val.astype(bf)
            def at_time(v, t):
                t = max(0, min(t, last_k - PAD))
                ct, r = divmod(t, m0)
                r = r // PAD * PAD
                return v[r:r + PAD, ct * 512:ct * 512 + 128]
            h = None
            xk = []
            kx[0].wait(); issue(1)
            xk.append(x_v[0:ks[0], 0:m0].T)
            pin(w1_v, xk[0][pin0[0]:pin0[0] + PAD, :])
            kw[0].wait(); issue(1)
            for i in range(nk):
                p = jnp.dot(xk[i], w1_v[ko[i]:ko[i] + ks[i], 0:c0], preferred_element_type=jnp.float32)
                h = p if h is None else h + p
                if i + 1 < nk:
                    dur = last_k * (-(-ks[i] // 128))
                    pin(x_v, at_time(h, last_k - lkx))
                    kx[i + 1].wait(); issue(1)
                    xk.append(x_v[ko[i + 1]:ko[i + 1] + ks[i + 1], 0:m0].T)
                    pin(w1_v, at_time(h, last_k - lkw))
                    kw[i + 1].wait(); issue(1)
            x0 = jnp.concatenate(xk, axis=1)
            for q in range(0, m0, 128):
                xt[q] = x0[q:q + 128]
            av = silu_bf16(h)
            for s, t in place.get(-1, []):
                wait(s, at_time(av, t))
            a_v[0:m0, 0:c0] = av
            for i, (r0, r1, f0, f1) in enumerate(items):
                h = jnp.dot(xrows(r0, r1), w1_v[0:D, f0:f1], preferred_element_type=jnp.float32)
                av = silu_bf16(h)
                for s, t in place.get(i, []):
                    ct, r = divmod(t, r1 - r0)
                    r = r // PAD * PAD
                    wait(s, av[r:r + PAD, ct * 128:(ct + 1) * 128])
                a_v[r0:r1, f0:f1] = av
        if scoped:
            pl.run_scoped(phase1, pltpu.SemaphoreType.DMA((ns + 1 + 2 * nk,)))
        else:
            phase1(sc[no + 1])
        ocp = [pltpu.make_async_copy(o_v[k], oT_hbm.at[pl.ds(r0, r1 - r0), pl.ds(a, b - a)], sem_out.at[0])
               for k, (a, b, r0, r1) in enumerate(outs)]
        for k, (a, b, r0, r1) in enumerate(outs):
            o = lax.dot_general(w2_v[r0:r1, :], a_v[a:b, :], (((1,), (1,)), ((), ())), preferred_element_type=jnp.float32)
            o_v[k][...] = o.astype(bf)
            ocp[k].start()
        for c in ocp:
            c.wait()

    @jax.jit
    def f(x, w1, w2):
        B, S, _ = x.shape
        xT = x.reshape(B * S, D).T
        hbm = pl.BlockSpec(memory_space=pltpu.HBM)
        scratch = [pltpu.VMEM((D + PAD, M), bf), pltpu.VMEM((D + PAD, F), bf), pltpu.VMEM((D + PAD, F), bf), pltpu.VMEM((M, F), bf)]
        scratch += [pltpu.VMEM((r1 - r0, b - a), bf) for (a, b, r0, r1) in outs]
        scratch += [pltpu.SemaphoreType.DMA((1,))]
        if not scoped:
            scratch += [pltpu.SemaphoreType.DMA((ns + 1 + 2 * nk,))]
        out = pl.pallas_call(
            kern, in_specs=[hbm, hbm, hbm], out_specs=hbm,
            out_shape=jax.ShapeDtypeStruct((D, B * S), x.dtype),
            scratch_shapes=scratch,
            compiler_params=pltpu.CompilerParams(vmem_limit_bytes=100 * 1024 * 1024, flags=flags),
        )(xT, w1, w2.T)
        return out.T.reshape(B, S, D)
    return f


_impl = make()


@jax.jit
def pallas_standalone__dense_activation_silu__prompt_kernel(x, w1, w2):
    return _impl(x, w1, w2)
```

```python
import jax
import jax.numpy as jnp
from jax import lax
import jax.experimental.pallas as pl
import jax.experimental.pallas.tpu as pltpu

M, D, F = 2048, 448, 1792
TILE = 128
KT = D // TILE * TILE
PAD = 16
ROWS = 512
COLS = 512
X_PIECES = (512, 512, 1024)
OUT_BLOCKS = (
    (0, 512, 0, D), (512, 1024, 0, D), (1024, 1536, 0, D), (1536, 1792, 0, D),
    (1792, M, 0, 384), (1792, M, 384, D),
)
LEAD_W, LEAD_X, LEAD_X_LATE, LEAD_W2 = 208, 330, 2000, 4000


def _plan():
    copies, steps, first_use, lead = [], [], [], []

    def copy(array, r0, r1, c0, c1, cycles):
        copies.append((array, r0, r1, c0, c1))
        first_use.append(len(steps))
        lead.append(cycles)

    wide = F // COLS * COLS
    copy("x", KT, D, 0, ROWS, LEAD_X)
    for f in range(0, wide, COLS):
        copy("w1", KT, D, f, f + COLS, LEAD_W)
        steps.append((0, ROWS, KT, D, f, f + COLS))
    for k in range(0, KT, TILE):
        copy("x", k, k + TILE, 0, ROWS, LEAD_X)
        copy("w1", k, k + TILE, 0, COLS, LEAD_W)
        steps.append((0, ROWS, k, k + TILE, 0, COLS))
    for f in range(COLS, wide, COLS):
        copy("w1", 0, KT, f, f + COLS, LEAD_W)
        steps.append((0, ROWS, 0, KT, f, f + COLS))
    copy("w1", 0, D, wide, F, LEAD_W)
    steps.append((0, ROWS, 0, D, wide, F))
    m = X_PIECES[0]
    for n in X_PIECES[1:]:
        copy("x", 0, D, m, m + n, LEAD_X_LATE)
        for r in range(m, m + n, ROWS):
            steps.append((r, r + ROWS, 0, D, 0, F))
        m += n
    copy("w2", 0, D, 0, F, LEAD_W2)

    start = [0]
    for m0, m1, k0, k1, f0, f1 in steps:
        tiles = pl.cdiv(k1 - k0, TILE) * ((f1 - f0) // TILE)
        start.append(start[-1] + (m1 - m0) * tiles // 4)
    waits, last = {}, (-1, 0)
    for c in range(len(copies)):
        at = (-1, 0)
        if first_use[c] > 0:
            t = max(start[first_use[c]] - lead[c], 0)
            s = max(s for s in range(first_use[c]) if start[s] <= t)
            at = (s, t - start[s])
        last = max(last, at)
        waits.setdefault(last[0], []).append((c, last[1]))
    return copies, steps, waits


def _silu(h):
    g = 0.5 * h
    return g + g * jnp.tanh(g)


def _kernel(xT_hbm, w1_hbm, w2T_hbm, oT_hbm, x_v, w1_v, w2_v, a_v, out_sem, *o_v):
    copies, steps, waits = _plan()
    hbm = {"x": xT_hbm, "w1": w1_hbm, "w2": w2T_hbm}
    vmem = {"x": x_v, "w1": w1_v, "w2": w2_v}
    stores = [
        pltpu.make_async_copy(
            buf, oT_hbm.at[pl.ds(r0, r1 - r0), pl.ds(c0, c1 - c0)], out_sem.at[0])
        for buf, (c0, c1, r0, r1) in zip(o_v, OUT_BLOCKS)
    ]

    def compute(in_sems):
        loads = []
        for c, (array, r0, r1, c0, c1) in enumerate(copies):
            window = (pl.ds(r0, r1 - r0), pl.ds(c0, c1 - c0))
            loads.append(pltpu.make_async_copy(
                hbm[array].at[window], vmem[array].at[window], in_sems.at[c]))
        for load in loads:
            load.start()

        xts = {}

        def x_block(m0, k0, k1):
            pieces, k = [], k0
            while k < k1:
                if (m0, k) not in xts:
                    xts[m0, k] = x_v[k:k1, m0:m0 + ROWS].T
                pieces.append(xts[m0, k])
                k += pieces[-1].shape[1]
            return pieces[0] if len(pieces) == 1 else jnp.concatenate(pieces, axis=1)

        def wait(c, after):
            if after is not None:
                buf = vmem[copies[c][0]]
                buf[D:D + PAD, 0:after.shape[1]] = after.astype(buf.dtype)
            loads[c].wait()

        after = None
        for c, _ in waits[-1]:
            wait(c, after)
            if copies[c][0] == "x":
                after = x_block(0, KT, D)[0:PAD, :]

        partial = {}
        for s, (m0, m1, k0, k1, f0, f1) in enumerate(steps):
            h = jnp.dot(x_block(m0, k0, k1), w1_v[k0:k1, f0:f1],
                        preferred_element_type=jnp.float32)
            done = k1 - k0
            if (m0, f0) in partial:
                h_prev, done_prev = partial.pop((m0, f0))
                h, done = h + h_prev, done + done_prev
            if done == D:
                h = _silu(h).astype(a_v.dtype)
            else:
                partial[m0, f0] = (h, done)
            for c, cycle in waits.get(s, []):
                turn, row = divmod(cycle, m1 - m0)
                col = min(turn * 4 // pl.cdiv(k1 - k0, TILE), (f1 - f0) // TILE - 1) * TILE
                row = row // PAD * PAD
                wait(c, h[row:row + PAD, col:col + TILE])
            if done == D:
                a_v[m0:m1, f0:f1] = h

        for buf, store, (c0, c1, r0, r1) in zip(o_v, stores, OUT_BLOCKS):
            out = lax.dot_general(w2_v[r0:r1, :], a_v[c0:c1, :], (((1,), (1,)), ((), ())),
                                  preferred_element_type=jnp.float32)
            buf[...] = out.astype(buf.dtype)
            store.start()

    pl.run_scoped(compute, pltpu.SemaphoreType.DMA((len(copies),)))
    for store in stores:
        store.wait()


@jax.jit
def pallas_standalone__dense_activation_silu__prompt_kernel(
    x: jax.Array,
    w1: jax.Array,
    w2: jax.Array,
):
    assert x.shape == (1, M, D) and w1.shape == (D, F) and w2.shape == (F, D)
    hbm = pl.BlockSpec(memory_space=pltpu.HBM)
    scratch = [
        pltpu.VMEM((D + PAD, M), x.dtype),
        pltpu.VMEM((D + PAD, F), w1.dtype),
        pltpu.VMEM((D + PAD, F), w2.dtype),
        pltpu.VMEM((M, F), x.dtype),
        pltpu.SemaphoreType.DMA((1,)),
    ] + [pltpu.VMEM((r1 - r0, c1 - c0), x.dtype) for c0, c1, r0, r1 in OUT_BLOCKS]
    outT = pl.pallas_call(
        _kernel,
        in_specs=[hbm, hbm, hbm],
        out_specs=hbm,
        out_shape=jax.ShapeDtypeStruct((D, M), x.dtype),
        scratch_shapes=scratch,
        compiler_params=pltpu.CompilerParams(
            vmem_limit_bytes=64 * 1024 * 1024,
            flags={"XLA_TPU_RESCHEDULE_DMA_DONES": True},
        ),
    )(x.reshape(M, D).T, w1, w2.T)
    return outT.T.reshape(1, M, D)
```
